```python
import jax
import jax.numpy as jnp

def _softmax(x, axis=-1):
    return jax.nn.softmax(x, axis=axis)

def _gelu(x):
    return jax.nn.gelu(x, approximate=True)

def _silu(x):
    return jax.nn.silu(x)

def _sigmoid(x):
    return jax.nn.sigmoid(x)

def _layernorm(x, axis=-1, eps=1e-05):
    m = jnp.mean(x, axis=axis, keepdims=True)
    v = jnp.var(x, axis=axis, keepdims=True)
    return (x - m) / jnp.sqrt(v + eps)

def _scatter_add(tgt, idx, src, axis=0):
    return tgt.at[idx].add(src)

def _segment_sum(src, seg, n):
    return jax.ops.segment_sum(src, seg, n)

class _Rng:

    def __init__(self, key):
        self._k = key

    def _next(self):
        self._k, sub = jax.random.split(self._k)
        return sub

    def normal(self, shape):
        return jax.random.normal(self._next(), shape, dtype=jnp.bfloat16)

    def randint(self, lo, hi, shape):
        return jax.random.randint(self._next(), shape, lo, hi, dtype=jnp.int32)

    def uniform(self, shape, lo=0.0, hi=1.0):
        return jax.random.uniform(self._next(), shape, jnp.bfloat16, lo, hi)

    def permutation(self, n):
        return jax.random.permutation(self._next(), n)
kernel_name = 'adaLN_cond__memory_aug_recurrent_mem_tr__dense_activation_gelu__prompt'

def setup_inputs():
    _rng = _Rng(jax.random.key(int.from_bytes(__import__("os").urandom(4), "little")))
    _w = lambda a: (lambda t: t.astype(jnp.bfloat16) if jnp.issubdtype(t.dtype, jnp.floating) else t)(jnp.asarray(a))

    def _A_setup():
        B, S, Dm = (1, 2048, 1024)
        H, Dh = (32, 128)
        M, seg = (8, 32)
        seg = min(seg, S)
        S = S // seg * seg
        return {'x': _w((lambda *s: _rng.normal(s) * 0.05)(B, S, Dm)), 'mem0': _w((lambda *s: _rng.normal(s) * 0.05)(B, M, Dm)), 'Wq': _w((lambda *s: _rng.normal(s) * 0.05)(Dm, H, Dh) * Dm ** (-0.5)), 'Wk': _w((lambda *s: _rng.normal(s) * 0.05)(Dm, H, Dh) * Dm ** (-0.5)), 'Wv': _w((lambda *s: _rng.normal(s) * 0.05)(Dm, H, Dh) * Dm ** (-0.5)), 'Wo': _w((lambda *s: _rng.normal(s) * 0.05)(H, Dh, Dm) * (H * Dh) ** (-0.5)), 'seg_len': seg}
    _A_in = _A_setup()

    def _B_setup():
        B, S, D, F = (1, 2048, 1024, 3584)
        return {'x': _w((lambda *s: _rng.normal(s) * 0.05)(B, S, D)), 'w1': _w((lambda *s: _rng.normal(s) * 0.05)(D, F) * D ** (-0.5)), 'b1': _w((lambda *s: _rng.normal(s) * 0.05)(F) * 0.01), 'w2': _w((lambda *s: _rng.normal(s) * 0.05)(F, D) * F ** (-0.5)), 'b2': _w((lambda *s: _rng.normal(s) * 0.05)(D) * 0.01)}
    _B_in = _B_setup()
    return {'A_x': _A_in['x'], 'A_mem0': _A_in['mem0'], 'A_Wq': _A_in['Wq'], 'A_Wk': _A_in['Wk'], 'A_Wv': _A_in['Wv'], 'A_Wo': _A_in['Wo'], 'A_seg_len': _A_in['seg_len'], 'B_x': _B_in['x'], 'B_w1': _B_in['w1'], 'B_b1': _B_in['b1'], 'B_w2': _B_in['w2'], 'B_b2': _B_in['b2'], 'c': _w((lambda *s: _rng.normal(s) * 0.05)(1, 1024)), 'w_mod': _w((lambda *s: _rng.normal(s) * 0.05)(1024, 6 * 1024) * 1024 ** (-0.5))}

def reference(A_x, A_mem0, A_Wq, A_Wk, A_Wv, A_Wo, A_seg_len, B_x, B_w1, B_b1, B_w2, B_b2, c, w_mod):

    def _A_ref(x, mem0, Wq, Wk, Wv, Wo, seg_len):
        B, S, Dm = x.shape
        H, Dh = (Wq.shape[1], Wq.shape[2])
        M = mem0.shape[1]
        scale = Dh ** (-0.5)
        n_seg = S // seg_len
        L = M + seg_len
        idx = jnp.arange(L)
        mask = (idx[:, None] < M) | (idx[:, None] >= idx[None, :])
        mem = mem0
        outs = []
        for s in range(n_seg):
            xs = x[:, s * seg_len:(s + 1) * seg_len, :].copy()
            h = jnp.concatenate([mem, xs], axis=1)
            q = jnp.einsum('btd,dhe->bhte', h, Wq)
            k = jnp.einsum('btd,dhe->bhte', h, Wk)
            v = jnp.einsum('btd,dhe->bhte', h, Wv)
            scores = jnp.einsum('bhqe,bhke->bhqk', q, k) * scale
            scores = jnp.where(mask[None, None], scores, -1000000000.0)
            p = _softmax(scores, axis=-1)
            o = jnp.einsum('bhqk,bhke->bhqe', p, v)
            o = jnp.einsum('bhte,hed->btd', o, Wo)
            mem = o[:, :M, :].copy()
            outs.append(o[:, M:, :])
        return jnp.concatenate(outs, axis=1)

    def _B_ref(x, w1, b1, w2, b2):
        h = jnp.einsum('bsd,df->bsf', x, w1) + b1
        h = _gelu(h)
        return jnp.einsum('bsf,fd->bsd', h, w2) + b2
    x = A_x
    mod = (_silu(c) @ w_mod).reshape(c.shape[0], 6, 1, -1)
    sa, ca, ga, sb, cb, gb = (mod[:, 0].copy(), mod[:, 1].copy(), mod[:, 2].copy(), mod[:, 3].copy(), mod[:, 4].copy(), mod[:, 5].copy())
    h = _layernorm(x, axis=-1) * (1 + ca) + sa
    x = x + ga * _A_ref(h, A_mem0, A_Wq, A_Wk, A_Wv, A_Wo, A_seg_len)
    h = _layernorm(x, axis=-1) * (1 + cb) + sb
    x = x + gb * _B_ref(h, B_w1, B_b1, B_w2, B_b2)
    return x
```

```python
import functools
import jax
import jax.numpy as jnp
import numpy as np
from jax import lax
import jax.experimental.pallas as pl
import jax.experimental.pallas.tpu as pltpu

F32 = jnp.float32
BF16 = jnp.bfloat16
U32 = jnp.uint32


def _bf(w_u32):
    return pltpu.bitcast(w_u32, BF16)


def _dot(a, b):
    return jnp.dot(a, b, preferred_element_type=F32)


def _kernel(x_hbm, mem0_ref, wq_hbm, wk_hbm, wv_hbm, wo_hbm, w1_hbm, b1_ref, w2_hbm, b2_ref,
            c_ref, wmod_hbm, out_ref,
            xv, wq, wk, wv, wo, w1, w2, wmod, stage, sems,
            *, S, D, H, E, M, SEG, F, G):
    n_seg = S // SEG
    L = M + SEG

    def cp(src, dst, i):
        return pltpu.make_async_copy(src, dst, sems.at[i])

    c_wmod = cp(wmod_hbm.bitcast(U32), wmod, 0)
    c_x = cp(x_hbm, xv, 1)
    c_q = cp(wq_hbm.bitcast(U32), stage.at[0], 2)
    c_k = cp(wk_hbm.bitcast(U32), stage.at[1], 3)
    c_v = cp(wv_hbm.bitcast(U32), stage.at[0], 4)
    c_o = cp(wo_hbm.bitcast(U32), wo, 5)
    c_1 = cp(w1_hbm.bitcast(U32), w1, 6)
    c_2 = cp(w2_hbm.bitcast(U32), w2, 7)
    c_q.start(); c_k.start(); c_wmod.start(); c_x.start()

    def relayout(slot, dst):
        HP = H // 2

        def body(j, _):
            base = j * (16 * HP)
            r = pl.ds(pl.multiple_of(j * 8, 8), 8)
            for p in range(HP):
                a = stage[slot, pl.ds(base + p, 8, stride=2 * HP), :]
                b = stage[slot, pl.ds(base + HP + p, 8, stride=2 * HP), :]
                dst[r, (2 * p) * E:(2 * p + 1) * E] = (a & U32(0xffff)) | (b << 16)
                dst[r, (2 * p + 1) * E:(2 * p + 2) * E] = (a >> 16) | (b & U32(0xffff0000))
            return 0
        lax.fori_loop(0, D // 16, body, 0)

    c_q.wait(); relayout(0, wq)
    c_v.start(); c_o.start(); c_1.start(); c_2.start()
    c_k.wait(); relayout(1, wk)
    c_wmod.wait()
    cc = c_ref[...].astype(F32)
    sc = cc * jax.nn.sigmoid(cc)
    mod = _dot(jnp.broadcast_to(sc, (8, D)).astype(BF16), _bf(wmod[...]))[0:1, :]
    sa, ca, ga, sb, cb, gb = [mod[:, i * D:(i + 1) * D] for i in range(6)]
    c_x.wait()
    c_v.wait(); relayout(0, wv)
    c_o.wait(); c_1.wait(); c_2.wait()

    row = lax.broadcasted_iota(jnp.int32, (L, L), 0)
    col = lax.broadcasted_iota(jnp.int32, (L, L), 1)
    mask = (row < M) | (row >= col)
    scale = float(E) ** -0.5
    b1 = b1_ref[...].astype(F32)
    b2 = b2_ref[...].astype(F32)

    def ln(x):
        m = jnp.mean(x, axis=-1, keepdims=True)
        xc = x - m
        v = jnp.mean(xc * xc, axis=-1, keepdims=True)
        return xc * lax.rsqrt(v + 1e-5)

    def step(s, mem):
        r = pl.ds(pl.multiple_of(s * SEG, SEG), SEG)
        x = xv[r, :].astype(F32)
        h = ln(x) * (1.0 + ca) + sa
        hc = jnp.concatenate([mem, h], axis=0)
        outs = []
        for g in range(H // G):
            cs = slice(g * G * E, (g + 1) * G * E)
            q = _dot(hc, _bf(wq[:, cs]))
            k = _dot(hc, _bf(wk[:, cs]))
            v = _dot(hc, _bf(wv[:, cs]))
            for j in range(G):
                js = slice(j * E, (j + 1) * E)
                sco = lax.dot_general(q[:, js], k[:, js].astype(BF16), (((1,), (1,)), ((), ())),
                                      preferred_element_type=F32) * scale
                sco = jnp.where(mask, sco, -1e9)
                p = jnp.exp(sco - jnp.max(sco, axis=-1, keepdims=True))
                l = jnp.sum(p, axis=-1, keepdims=True)
                o = _dot(p, v[:, js].astype(BF16))
                outs.append(o * (1.0 / l))
        o_all = jnp.concatenate(outs, axis=1)
        y = _dot(o_all, _bf(wo[...]))
        x1 = x + ga * y[M:, :]
        h2 = ln(x1) * (1.0 + cb) + sb
        u = _dot(h2, _bf(w1[...])) + b1
        u = jax.nn.gelu(u, approximate=True)
        z = _dot(u, _bf(w2[...])) + b2
        out_ref[r, :] = (x1 + gb * z).astype(out_ref.dtype)
        return y[:M, :]

    lax.fori_loop(0, n_seg, step, mem0_ref[...].astype(F32))


@functools.partial(jax.jit, static_argnames=("A_seg_len",))
def pallas_adaLN_cond__memory_aug_recurrent_mem_tr__dense_activation_gelu__prompt_kernel(
        A_x, A_mem0, A_Wq, A_Wk, A_Wv, A_Wo, A_seg_len, B_x, B_w1, B_b1, B_w2, B_b2, c, w_mod):
    B, S, D = A_x.shape
    _, H, E = A_Wq.shape
    M = A_mem0.shape[1]
    F = B_w1.shape[1]
    SEG = int(A_seg_len)
    assert B == 1
    any_spec = pl.BlockSpec(memory_space=pl.ANY)
    vm = pl.BlockSpec(memory_space=pltpu.VMEM)
    kern = functools.partial(_kernel, S=S, D=D, H=H, E=E, M=M, SEG=SEG, F=F, G=4)
    out = pl.pallas_call(
        kern,
        out_shape=jax.ShapeDtypeStruct((S, D), A_x.dtype),
        in_specs=[any_spec, vm, any_spec, any_spec, any_spec, any_spec, any_spec, vm, any_spec, vm, vm, any_spec],
        out_specs=vm,
        scratch_shapes=[
            pltpu.VMEM((S, D), BF16),
            pltpu.VMEM((D // 2, H * E), U32),
            pltpu.VMEM((D // 2, H * E), U32),
            pltpu.VMEM((D // 2, H * E), U32),
            pltpu.VMEM((H * E // 2, D), U32),
            pltpu.VMEM((D // 2, F), U32),
            pltpu.VMEM((F // 2, D), U32),
            pltpu.VMEM((D // 2, 6 * D), U32),
            pltpu.VMEM((2, D * H // 2, E), U32),
            pltpu.SemaphoreType.DMA((8,)),
        ],
        compiler_params=pltpu.CompilerParams(vmem_limit_bytes=110 * 2 ** 20),
    )(A_x.reshape(S, D), A_mem0.reshape(M, D), A_Wq.reshape(D * H, E), A_Wk.reshape(D * H, E),
      A_Wv.reshape(D * H, E), A_Wo.reshape(H * E, D), B_w1, B_b1.reshape(1, F), B_w2, B_b2.reshape(1, D),
      c, w_mod)
    return out.reshape(B, S, D)
```

```python
import functools
import jax
import jax.numpy as jnp
import numpy as np
from jax import lax
import jax.experimental.pallas as pl
import jax.experimental.pallas.tpu as pltpu

F32 = jnp.float32
BF16 = jnp.bfloat16
U32 = jnp.uint32


def _bf(w_u32):
    return pltpu.bitcast(w_u32, BF16)


def _dot(a, b):
    return jnp.dot(a, b, preferred_element_type=F32)


def _kernel(x_hbm, mem0_ref, wq_hbm, wk_hbm, wv_hbm, wo_hbm, w1_hbm, b1_ref, w2_hbm, b2_ref,
            c_ref, wmod_hbm, out_hbm,
            xv, outv, yv, hv, h2v, zv, wq, wk, wv, wo, w1, w2, wmod, modv, stage, sems, osems, wsems,
            *, S, D, H, E, M, SEG, F, cfg):
    n_seg = S // SEG
    L = M + SEG
    G = cfg["G"]; K = cfg["K"]; FC = cfg["FC"]

    def cp(src, dst, i):
        return pltpu.make_async_copy(src, dst, sems.at[i])

    wm = wmod_hbm.bitcast(U32)
    c_m0 = cp(wm.at[:, 0:2 * D], wmod.at[:, 0:2 * D], 0)
    c_m1 = cp(wm.at[:, 2 * D:6 * D], wmod.at[:, 2 * D:6 * D], 8)
    c_x = cp(x_hbm.at[0:256, :], xv.at[0:256, :], 1)
    c_x2 = cp(x_hbm.at[256:S, :], xv.at[256:S, :], 2)
    NC = cfg["NC"]
    CR = D * H // 2 // NC
    def wcp(w_hbm, slot, i):
        rows = pl.ds(i * CR, CR)
        return pltpu.make_async_copy(w_hbm.bitcast(U32).at[rows, :], stage.at[slot, rows, :], wsems.at[slot * NC + i])
    c_o = cp(wo_hbm.bitcast(U32), wo, 5)
    c_1 = cp(w1_hbm.bitcast(U32), w1, 6)
    c_2 = cp(w2_hbm.bitcast(U32), w2, 7)

    def relayout(slot, dst, i):
        HP = H // 2

        def body(j, _):
            base = j * (16 * HP)
            r = pl.ds(pl.multiple_of(j * 8, 8), 8)
            for p in range(HP):
                a = stage[slot, pl.ds(base + p, 8, stride=2 * HP), :]
                b = stage[slot, pl.ds(base + HP + p, 8, stride=2 * HP), :]
                dst[r, (2 * p) * E:(2 * p + 1) * E] = (a & U32(0xffff)) | (b << 16)
                dst[r, (2 * p + 1) * E:(2 * p + 2) * E] = (a >> 16) | (b & U32(0xffff0000))
            return 0
        n = D // 16 // NC
        lax.fori_loop(i * n, (i + 1) * n, body, 0)

    ws = [(wq_hbm, wq), (wk_hbm, wk), (wv_hbm, wv)]
    items = [(t, i) for t in range(3) for i in range(NC)]
    AH = cfg["AH"]
    c_m0.start(); c_x.start()
    for (t, i) in items[:AH]:
        wcp(ws[t][0], t, i).start()
    for n_, (t, i) in enumerate(items):
        wcp(ws[t][0], t, i).wait()
        if n_ + AH < len(items):
            t2, i2 = items[n_ + AH]
            wcp(ws[t2][0], t2, i2).start()
        elif n_ + AH == len(items):
            c_o.start()
        relayout(t, ws[t][1], i)
        if n_ == 2:
            c_m0.wait()
            cc = c_ref[...].astype(F32)
            sc = jnp.broadcast_to(cc * jax.nn.sigmoid(cc), (8, D)).astype(BF16)
            modv[:, 0:2 * D] = _dot(sc, _bf(wmod[:, 0:2 * D]))
            c_x.wait()
    c_x2.start(); c_m1.start(); c_1.start(); c_2.start()

    row = lax.broadcasted_iota(jnp.int32, (L, L), 0)
    col = lax.broadcasted_iota(jnp.int32, (L, L), 1)
    mask = (row < M) | (row >= col)
    scale = float(E) ** -0.5

    def ln(x):
        m = jnp.mean(x, axis=-1, keepdims=True)
        xc = x - m
        v = jnp.mean(xc * xc, axis=-1, keepdims=True)
        return xc * lax.rsqrt(v + 1e-5)

    def modrow(i):
        return modv[0:1, i * D:(i + 1) * D]

    def ffn_pre(r):
        x1 = xv[r, :].astype(F32) + modrow(2) * yv[r, :]
        h2 = ln(x1) * (1.0 + modrow(4)) + modrow(3)
        return x1, h2

    def ffn_chunk(h2, ci, z):
        cs = slice(ci * FC, (ci + 1) * FC)
        u = _dot(h2, _bf(w1[:, cs])) + b1_ref[:, cs].astype(F32)
        u = jax.nn.gelu(u, approximate=True)
        zz = _dot(u, _bf(w2[ci * FC // 2:(ci + 1) * FC // 2, :]))
        return zz if z is None else z + zz

    def ffn_post(r, x1, z):
        outv[r, :] = (x1 + modrow(5) * (z + b2_ref[...].astype(F32))).astype(outv.dtype)

    def seg(i):
        return pl.ds(pl.multiple_of(i * SEG, SEG), SEG)

    def mk_h(i):
        hv[seg(i), :] = (ln(xv[seg(i), :].astype(F32)) * (1.0 + modrow(1)) + modrow(0)).astype(BF16)

    def mk_h2(i):
        h2v[...] = ffn_pre(seg(i))[1]

    def step(s, mem, do_ffn, last=False):
        hc = jnp.concatenate([mem, hv[seg(s), :].astype(F32)], axis=0)
        ng = H // G
        nch = F // FC
        st = {}
        if do_ffn:
            h2 = h2v[...]

        def P(g):
            cs = slice(g * G * E, (g + 1) * G * E)
            st["q", g] = _dot(hc, _bf(wq[:, cs]))
            st["k", g] = _dot(hc, _bf(wk[:, cs])).astype(BF16)
            st["v", g] = _dot(hc, _bf(wv[:, cs])).astype(BF16)

        def Sc(g):
            ps = []
            for j in range(G):
                js = slice(j * E, (j + 1) * E)
                sco = lax.dot_general(st["q", g][:, js], st["k", g][:, js], (((1,), (1,)), ((), ())),
                                      preferred_element_type=F32) * scale
                sco = jnp.where(mask, sco, -1e9)
                p = jnp.exp(sco - jnp.max(sco, axis=-1, keepdims=True))
                ps.append((p, jnp.sum(p, axis=-1, keepdims=True)))
            st["p", g] = ps

        def V(g):
            os_ = []
            for j in range(G):
                js = slice(j * E, (j + 1) * E)
                p, l = st["p", g][j]
                os_.append(_dot(p, st["v", g][:, js]) * pl.reciprocal(l, approx=False))
            st["o", g] = jnp.concatenate(os_, axis=1)

        def O(g):
            yy = _dot(st["o", g], _bf(wo[g * G * E // 2:(g + 1) * G * E // 2, :]))
            st["y"] = yy if "y" not in st else st["y"] + yy

        def F1(c):
            if not do_ffn or c >= nch: return
            cs = slice(c * FC, (c + 1) * FC)
            u = _dot(h2, _bf(w1[:, cs])) + b1_ref[:, cs].astype(F32)
            st["u", c] = jax.nn.gelu(u, approximate=True)

        def F2(c):
            if not do_ffn or c >= nch or c < 0: return
            zz = _dot(st["u", c], _bf(w2[c * FC // 2:(c + 1) * FC // 2, :]))
            st["z"] = zz if "z" not in st else st["z"] + zz

        P(0)
        F1(0)
        for g in range(ng):
            if g + 1 < ng:
                P(g + 1)
            Sc(g)
            if g >= 1 and do_ffn:
                O(g - 1)
            F1(g + 1)
            if g < nch - 2:
                F2(g)
            if g == 1 and do_ffn:
                post(s - K - 1, s > K)
            if g == 2:
                mk_h(jnp.minimum(s + 1, n_seg - 1))
            if g == 4 and do_ffn:
                mk_h2(s + 1 - K)
            V(g)
        F2(nch - 2)
        if not do_ffn:
            pl.when(s == 0)(lambda: c_o.wait())
            for g in range(ng - 1):
                O(g)
        O(ng - 1)
        F2(nch - 1)
        y = st["y"]
        yv[seg(s), :] = y[M:, :]
        if do_ffn:
            zv[...] = st["z"]
        return y[:M, :]

    def post(i, cond=None):
        rf = seg(jnp.maximum(i, 0))
        x1 = xv[rf, :].astype(F32) + modrow(2) * yv[rf, :]
        ffn_post(rf, x1, zv[...])

    mk_h(0)
    mem = lax.fori_loop(0, K, functools.partial(step, do_ffn=False), mem0_ref[...].astype(F32))
    c_x2.wait(); c_m1.wait(); c_1.wait(); c_2.wait()
    modv[:, 2 * D:6 * D] = _dot(sc, _bf(wmod[:, 2 * D:6 * D]))
    mk_h2(0)
    zv[...] = jnp.zeros(zv.shape, F32)
    OC = cfg["OC"]
    def out_cp(i):
        rows = pl.ds(i * (S // OC), S // OC)
        return pltpu.make_async_copy(outv.at[rows, :], out_hbm.at[rows, :], osems.at[i])
    spc = n_seg // OC
    def step2(s, mem):
        mem = step(s, mem, True)
        for i in range(OC - 1):
            @pl.when(s - K == (i + 1) * spc)
            def _():
                out_cp(i).start()
        return mem
    lax.fori_loop(K, cfg.get("nst", n_seg), step2, mem)
    post(n_seg - K - 1)
    rt = pl.ds((n_seg - K) * SEG, K * SEG)
    x1, h2 = ffn_pre(rt)
    z = None
    for ci in range(F // FC):
        z = ffn_chunk(h2, ci, z)
    ffn_post(rt, x1, z)
    out_cp(OC - 1).start()
    for i in range(OC):
        out_cp(i).wait()


@functools.partial(jax.jit, static_argnames=("A_seg_len",))
def pallas_adaLN_cond__memory_aug_recurrent_mem_tr__dense_activation_gelu__prompt_kernel(
        A_x, A_mem0, A_Wq, A_Wk, A_Wv, A_Wo, A_seg_len, B_x, B_w1, B_b1, B_w2, B_b2, c, w_mod):
    cfg = dict(G=4, K=5, FC=512, OC=8, NC=4, AH=3)
    B, S, D = A_x.shape
    _, H, E = A_Wq.shape
    M = A_mem0.shape[1]
    F = B_w1.shape[1]
    SEG = int(A_seg_len)
    assert B == 1
    any_spec = pl.BlockSpec(memory_space=pl.ANY)
    vm = pl.BlockSpec(memory_space=pltpu.VMEM)
    kern = functools.partial(_kernel, S=S, D=D, H=H, E=E, M=M, SEG=SEG, F=F, cfg=cfg)
    out = pl.pallas_call(
        kern,
        out_shape=jax.ShapeDtypeStruct((S, D), A_x.dtype),
        in_specs=[any_spec, vm, any_spec, any_spec, any_spec, any_spec, any_spec, vm, any_spec, vm, vm, any_spec],
        out_specs=any_spec,
        scratch_shapes=[
            pltpu.VMEM((S, D), BF16),
            pltpu.VMEM((S, D), BF16),
            pltpu.VMEM((S, D), F32),
            pltpu.VMEM((S, D), BF16),
            pltpu.VMEM((SEG, D), F32),
            pltpu.VMEM((SEG, D), F32),
            pltpu.VMEM((D // 2, H * E), U32),
            pltpu.VMEM((D // 2, H * E), U32),
            pltpu.VMEM((D // 2, H * E), U32),
            pltpu.VMEM((H * E // 2, D), U32),
            pltpu.VMEM((D // 2, F), U32),
            pltpu.VMEM((F // 2, D), U32),
            pltpu.VMEM((D // 2, 6 * D), U32),
            pltpu.VMEM((8, 6 * D), F32),
            pltpu.VMEM((3, D * H // 2, E), U32),
            pltpu.SemaphoreType.DMA((9,)),
            pltpu.SemaphoreType.DMA((cfg["OC"],)),
            pltpu.SemaphoreType.DMA((3 * cfg["NC"],)),
        ],
        compiler_params=pltpu.CompilerParams(vmem_limit_bytes=122 * 2 ** 20, **cfg.get("cp", {})),
    )(A_x.reshape(S, D), A_mem0.reshape(M, D), A_Wq.reshape(D * H, E), A_Wk.reshape(D * H, E),
      A_Wv.reshape(D * H, E), A_Wo.reshape(H * E, D), B_w1, B_b1.reshape(1, F), B_w2, B_b2.reshape(1, D),
      c, w_mod)
    return out.reshape(B, S, D)
```
